```python
import os as _os
_os.environ.setdefault("JAX_PLATFORMS", "cpu")
import jax
import jax.numpy as jnp

def _softmax(x, axis=-1):
    return jax.nn.softmax(x, axis=axis)
def _gelu(x):
    return jax.nn.gelu(x, approximate=True)
def _silu(x):
    return jax.nn.silu(x)
def _sigmoid(x):
    return jax.nn.sigmoid(x)
def _layernorm(x, axis=-1, eps=1e-5):
    m = jnp.mean(x, axis=axis, keepdims=True)
    v = jnp.var(x, axis=axis, keepdims=True)
    return (x - m) / jnp.sqrt(v + eps)
def _scatter_add(tgt, idx, src, axis=0):
    return tgt.at[idx].add(src)
def _segment_sum(src, seg, n):
    return jax.ops.segment_sum(src, seg, n)
class _Rng:
    def __init__(self, key):
        self._k = key
    def _next(self):
        self._k, sub = jax.random.split(self._k)
        return sub
    def normal(self, shape):
        return jax.random.normal(self._next(), shape, dtype=jnp.bfloat16)
    def randint(self, lo, hi, shape):
        return jax.random.randint(self._next(), shape, lo, hi, dtype=jnp.int32)
    def uniform(self, shape, lo=0.0, hi=1.0):
        return jax.random.uniform(self._next(), shape, jnp.bfloat16, lo, hi)
    def permutation(self, n):
        return jax.random.permutation(self._next(), n)


kernel_name = 'parallel_sum__sliding_block__moe_arch_mod__prompt'

def setup_inputs():
    _rng = _Rng(jax.random.key(int.from_bytes(__import__("os").urandom(4), "little")))
    _w = (lambda a: (lambda t: t.astype(jnp.bfloat16) if jnp.issubdtype(t.dtype, jnp.floating) else t)(jnp.asarray(a)))
    def _A_setup():
        B, S, D = 1, 2048, 512
        return {
            "x": _w((lambda *s: _rng.normal(s) * 0.05)(B, S, D)),
            "wqkv": _w((lambda *s: _rng.normal(s) * 0.05)(D, 3 * D)),
            "wo": _w((lambda *s: _rng.normal(s) * 0.05)(D, D)),
        }
    _A_in = _A_setup()

    def _B_setup():
        B, S, D, F, C = 1, 2048, 512, 1376, 1
        return {
            "x": _w((lambda *s: _rng.normal(s) * 0.05)(B, S, D)),
            "w_r": _w((lambda *s: _rng.normal(s) * 0.05)(D)),
            "w_gate": _w((lambda *s: _rng.normal(s) * 0.05)(D, F)),
            "w_up": _w((lambda *s: _rng.normal(s) * 0.05)(D, F)),
            "w_down": _w((lambda *s: _rng.normal(s) * 0.05)(F, D)),
        }
    _B_in = _B_setup()

    return {
        "A_x": _A_in["x"],
        "A_wqkv": _A_in["wqkv"],
        "A_wo": _A_in["wo"],
        "B_x": _B_in["x"],
        "B_w_r": _B_in["w_r"],
        "B_w_gate": _B_in["w_gate"],
        "B_w_up": _B_in["w_up"],
        "B_w_down": _B_in["w_down"],
    }

def reference(A_x, A_wqkv, A_wo, B_x, B_w_r, B_w_gate, B_w_up, B_w_down):
    def _A_ref(x, wqkv, wo):
        B, S, D = x.shape
        H = 32; Dh = D // H; W = 256
        qkv = (lambda x, *d: x.transpose(*d))((x @ wqkv).reshape(B, S, 3, H, Dh), 2, 0, 3, 1, 4)
        q, k, v = qkv[0], qkv[1], qkv[2]
        scores = jnp.einsum("bhqd,bhkd->bhqk", q, k) * (Dh ** -0.5)
        idx = jnp.arange(S)
        mask = (idx[:, None] - idx[None, :] >= 0) & (idx[:, None] - idx[None, :] < W)
        scores = jnp.where(mask[None, None], scores, -1e9)
        p = _softmax(scores, axis=-1)
        o = jnp.einsum("bhqk,bhkd->bhqd", p, v)
        return (lambda x, *d: x.transpose(*d))(o, 0, 2, 1, 3).reshape(B, S, D) @ wo

    def _B_ref(x, w_r, w_gate, w_up, w_down):
        B, S, D = x.shape
        C = 1
        r = x @ w_r
        idx = jnp.argsort(-r, axis=-1)[:, :C]
        idx_e = jnp.repeat(idx.reshape(B, C, 1), D, axis=2)
        x_sel = jnp.take_along_axis(x, idx_e, axis=1)
        g = _silu(x_sel @ w_gate)
        u = x_sel @ w_up
        y = (g * u) @ w_down
        r_sel = _sigmoid(jnp.take_along_axis(r, idx, axis=1))
        y = y * r_sel.reshape(B, C, 1)
        b_off = (jnp.arange(B) * S).reshape(B, 1)
        flat_idx = (idx + b_off).reshape(B * C)
        zero = (x * 0.0).reshape(B * S, D)
        upd = _scatter_add(zero, flat_idx, y.reshape(B * C, D), axis=0)
        return x + upd.reshape(B, S, D)

    x = A_x
    xn = _layernorm(x, axis=-1)
    return x + _A_ref(xn, A_wqkv, A_wo) + _B_ref(xn, B_w_r, B_w_gate, B_w_up, B_w_down)
```

```python
import jax
import jax.numpy as jnp
from jax import lax
import jax.experimental.pallas as pl
import jax.experimental.pallas.tpu as pltpu

S = 2048
D = 512
H = 32
DH = 16
W = 256
F = 1376
BQ = 128
NB = S // BQ
CH = 512
NC = S // CH
LN_EPS = 1e-5
NEG = -1e9
QSCALE = (DH ** -0.5) * 1.4426950408889634

_NT = (((1,), (1,)), ((), ()))
_NN = (((1,), (0,)), ((), ()))
_TN = (((0,), (0,)), ((), ()))


def _kernel(x_hbm, wqkv_hbm, wo_hbm, wr_ref, wg_hbm, wu_hbm, wd_hbm,
            o_ref,
            x_ref, wqkv_ref, wo_ref, wg_ref, wu_ref, wd_ref, wqt_s, wvt_s,
            xn_s, q_s, k_s, vt_s, y_s, ot_s, sa_s, sb_s, idx_s, sems):
    I = pl.program_id(0)
    f32 = jnp.float32
    bf16 = jnp.bfloat16

    @pl.when(I == 0)
    def _prologue():
        wr = wr_ref[...].astype(f32).reshape(1, D)

        def x_copy(c):
            r0 = pl.multiple_of(c * CH, CH)
            return pltpu.make_async_copy(x_hbm.at[pl.ds(r0, CH)], x_ref.at[pl.ds(r0, CH)],
                                         sems.at[c])
        def w_part(j):
            return pltpu.make_async_copy(wqkv_hbm.at[:, pl.ds(j * D, D)],
                                         wqkv_ref.at[:, pl.ds(j * D, D)], sems.at[NC + 5 + j])
        wo_cp = pltpu.make_async_copy(wo_hbm, wo_ref, sems.at[NC + 1])
        wg_cp = pltpu.make_async_copy(wg_hbm, wg_ref, sems.at[NC + 2])
        wu_cp = pltpu.make_async_copy(wu_hbm, wu_ref, sems.at[NC + 3])
        wd_cp = pltpu.make_async_copy(wd_hbm, wd_ref, sems.at[NC + 4])
        x_copy(0).start()
        w_part(1).start()
        w_part(0).start()
        w_part(2).start()
        for c in range(1, NC):
            x_copy(c).start()
        wo_cp.start()
        wg_cp.start()
        wu_cp.start()
        wd_cp.start()

        def ln_chunk(c, carry):
            best_val, best_idx = carry
            r0 = pl.multiple_of(c * CH, CH)
            xc = x_ref[pl.ds(r0, CH), :].astype(f32)
            m = jnp.mean(xc, axis=-1, keepdims=True)
            xc0 = xc - m
            v = jnp.mean(xc0 * xc0, axis=-1, keepdims=True)
            xn = (xc0 * lax.rsqrt(v + LN_EPS)).astype(bf16)
            xn_s[pl.ds(r0, CH), :] = xn
            r = jnp.sum(xn.astype(f32) * wr, axis=-1, keepdims=True)
            r = r.astype(bf16).astype(f32)
            cmax = jnp.max(r)
            rows = lax.broadcasted_iota(jnp.int32, (CH, 1), 0) + r0
            cidx = jnp.min(jnp.where(r == cmax, rows, S))
            better = cmax > best_val
            best_idx = jnp.where(better, cidx, best_idx)
            best_val = jnp.where(better, cmax, best_val)
            return best_val, best_idx

        def k_proj(c):
            r0 = pl.multiple_of(c * CH, CH)
            k = jnp.dot(xn_s[pl.ds(r0, CH), :], wqkv_ref[:, D:2 * D], preferred_element_type=f32)
            k_s[pl.ds(r0, CH), :] = k.astype(bf16)

        def qv_proj(c):
            r0 = pl.multiple_of(c * CH, CH)
            xn = xn_s[pl.ds(r0, CH), :]
            qt = lax.dot_general(wqt_s[...], xn, _NT, preferred_element_type=f32)
            q_s[:, pl.ds(r0, CH)] = (qt * QSCALE).astype(bf16)
            vt = lax.dot_general(wvt_s[...], xn, _NT, preferred_element_type=f32)
            vt_s[:, pl.ds(r0, CH)] = vt.astype(bf16)

        def proj_chunk(c):
            k_proj(c)
            qv_proj(c)

        x_copy(0).wait()
        best = ln_chunk(0, (jnp.float32(-jnp.inf), jnp.int32(0)))
        w_part(1).wait()
        k_proj(0)
        w_part(0).wait()
        w_part(2).wait()
        wqt_s[...] = wqkv_ref[:, 0:D].T
        wvt_s[...] = wqkv_ref[:, 2 * D:3 * D].T
        x_copy(1).wait()
        best = ln_chunk(1, best)
        qv_proj(0)

        def body(c, best):
            x_copy(c + 1).wait()
            best = ln_chunk(c + 1, best)
            proj_chunk(c)
            return best

        best_val, best_idx = lax.fori_loop(1, NC - 1, body, best)
        idx_s[0] = best_idx
        wo_cp.wait()
        wg_cp.wait()
        wu_cp.wait()
        wd_cp.wait()

        base = pl.multiple_of((best_idx // 16) * 16, 16)
        slab = xn_s[pl.ds(base, 16), :].astype(f32)
        rows16 = lax.broadcasted_iota(jnp.int32, (16, D), 0) + base
        xsel = jnp.sum(jnp.where(rows16 == best_idx, slab, 0.0), axis=0, keepdims=True)
        xsel8 = jnp.broadcast_to(xsel, (8, D)).astype(bf16)
        g = lax.dot_general(xsel8, wg_ref[...], _NT, preferred_element_type=f32)
        g = g.astype(bf16).astype(f32)
        g = (g * jax.nn.sigmoid(g)).astype(bf16).astype(f32)
        u = lax.dot_general(xsel8, wu_ref[...], _NT, preferred_element_type=f32)
        u = u.astype(bf16).astype(f32)
        hmid = (g * u).astype(bf16)
        y = jnp.dot(hmid, wd_ref[...], preferred_element_type=f32)
        y = y.astype(bf16).astype(f32)
        rsel = jax.nn.sigmoid(best_val).astype(bf16).astype(f32)
        y_s[...] = (y * rsel).astype(bf16).astype(f32)

        proj_chunk(NC - 1)

    r0 = pl.multiple_of(I * BQ, BQ)
    row = lax.broadcasted_iota(jnp.int32, (BQ, BQ), 0)
    col = lax.broadcasted_iota(jnp.int32, (BQ, BQ), 1)
    tri = row <= col

    def attention(ntiles):
        def koff(t):
            return pl.multiple_of((I - 2 + t) * BQ, BQ)

        def stage_a(j, sbuf):
            g, a0 = j // 2, (j % 2) * 4
            cols = []
            for u in range(4):
                a = a0 + u
                h = g * 8 + a
                parts = []
                if a > 0:
                    parts.append(jnp.zeros((a * DH, BQ), bf16))
                parts.append(q_s[pl.ds(h * DH, DH), pl.ds(r0, BQ)])
                if a < 7:
                    parts.append(jnp.zeros(((7 - a) * DH, BQ), bf16))
                cols.append(jnp.concatenate(parts, axis=0))
            wq = jnp.concatenate(cols, axis=1)
            ksl = lambda t: k_s[pl.ds(koff(t), BQ), g * 128:(g + 1) * 128]
            st2 = jnp.dot(ksl(2), wq, preferred_element_type=f32)
            st0 = jnp.dot(ksl(0), wq, preferred_element_type=f32) if ntiles == 3 else None
            ms = []
            for u in range(4):
                sl = slice(u * BQ, (u + 1) * BQ)
                other = st0[:, sl] if ntiles == 3 else NEG
                sm = jnp.where(tri, st2[:, sl], other)
                sbuf[0:BQ, sl] = sm
                ms.append(jnp.max(sm, axis=0, keepdims=True))
            m = jnp.concatenate(ms, axis=1)
            if ntiles >= 2:
                st1 = jnp.dot(ksl(1), wq, preferred_element_type=f32)
                sbuf[BQ:2 * BQ, :] = st1
                m = jnp.maximum(m, jnp.max(st1, axis=0, keepdims=True))
            return m

        def stage_b(j, sbuf, m):
            g, a0 = j // 2, (j % 2) * 4
            for u in range(4):
                h = g * 8 + a0 + u
                sl = slice(u * BQ, (u + 1) * BQ)
                mu = m[:, sl]
                vsl = lambda t: vt_s[pl.ds(h * DH, DH), pl.ds(koff(t), BQ)]
                pm = jnp.exp2(sbuf[0:BQ, sl] - mu)
                l = jnp.sum(pm, axis=0, keepdims=True)
                if ntiles == 3:
                    ot = jnp.dot(vsl(2), jnp.where(tri, pm, 0.0).astype(bf16),
                                 preferred_element_type=f32)
                    ot = ot + jnp.dot(vsl(0), jnp.where(tri, 0.0, pm).astype(bf16),
                                      preferred_element_type=f32)
                else:
                    ot = jnp.dot(vsl(2), pm.astype(bf16), preferred_element_type=f32)
                if ntiles >= 2:
                    p1 = jnp.exp2(sbuf[BQ:2 * BQ, sl] - mu)
                    l = l + jnp.sum(p1, axis=0, keepdims=True)
                    ot = ot + jnp.dot(vsl(1), p1.astype(bf16), preferred_element_type=f32)
                ot_s[pl.ds(h * DH, DH), :] = (ot / l).astype(bf16)

        bufs = (sa_s, sb_s)
        NQ = 8
        m_prev = stage_a(0, bufs[0])
        for j in range(NQ):
            m_next = stage_a(j + 1, bufs[(j + 1) % 2]) if j + 1 < NQ else None
            stage_b(j, bufs[j % 2], m_prev)
            m_prev = m_next

    @pl.when(I >= 2)
    def _():
        attention(3)

    @pl.when(I == 1)
    def _():
        attention(2)

    @pl.when(I == 0)
    def _():
        attention(1)

    att = lax.dot_general(ot_s[...], wo_ref[...], _TN,
                          preferred_element_type=f32)
    xb = x_ref[pl.ds(r0, BQ), :].astype(f32)
    xnb = xn_s[pl.ds(r0, BQ), :].astype(f32)
    rows = lax.broadcasted_iota(jnp.int32, (BQ, D), 0) + I * BQ
    upd = jnp.where(rows == idx_s[0], jnp.broadcast_to(y_s[0:1, :], (BQ, D)), 0.0)
    o_ref[...] = (xb + att + (xnb + upd)).astype(o_ref.dtype)


@jax.jit
def pallas_parallel_sum__sliding_block__moe_arch_mod__prompt_kernel(
    A_x: jax.Array,
    A_wqkv: jax.Array,
    A_wo: jax.Array,
    B_x: jax.Array,
    B_w_r: jax.Array,
    B_w_gate: jax.Array,
    B_w_up: jax.Array,
    B_w_down: jax.Array,
):
    del B_x
    x = A_x.reshape(S, D)
    wr = B_w_r
    bf16 = jnp.bfloat16
    f32 = jnp.float32
    any_spec = pl.BlockSpec(memory_space=pl.ANY)
    out = pl.pallas_call(
        _kernel,
        grid=(NB,),
        in_specs=[
            any_spec,
            any_spec,
            any_spec,
            pl.BlockSpec((D,), lambda i: (0,)),
            any_spec,
            any_spec,
            any_spec,
        ],
        out_specs=pl.BlockSpec((BQ, D), lambda i: (i, 0)),
        out_shape=jax.ShapeDtypeStruct((S, D), A_x.dtype),
        scratch_shapes=[
            pltpu.VMEM((S, D), bf16),
            pltpu.VMEM((D, 3 * D), bf16),
            pltpu.VMEM((D, D), bf16),
            pltpu.VMEM((F, D), bf16),
            pltpu.VMEM((F, D), bf16),
            pltpu.VMEM((F, D), bf16),
            pltpu.VMEM((D, D), bf16),
            pltpu.VMEM((D, D), bf16),
            pltpu.VMEM((S, D), bf16),
            pltpu.VMEM((D, S), bf16),
            pltpu.VMEM((S, D), bf16),
            pltpu.VMEM((D, S), bf16),
            pltpu.VMEM((8, D), f32),
            pltpu.VMEM((D, BQ), bf16),
            pltpu.VMEM((2 * BQ, 4 * BQ), f32),
            pltpu.VMEM((2 * BQ, 4 * BQ), f32),
            pltpu.SMEM((1,), jnp.int32),
            pltpu.SemaphoreType.DMA((NC + 8,)),
        ],
        compiler_params=pltpu.CompilerParams(
            dimension_semantics=("arbitrary",),
            vmem_limit_bytes=100 * 1024 * 1024,
        ),
    )(x, A_wqkv, A_wo, wr, B_w_gate.T, B_w_up.T, B_w_down)
    return out.reshape(A_x.shape)
```

```python
import jax
import jax.numpy as jnp
from jax import lax
import jax.experimental.pallas as pl
import jax.experimental.pallas.tpu as pltpu

S = 2048
D = 512
H = 32
DH = 16
W = 256
F = 1376
BQ = 128
NB = S // BQ
CH = 512
NC = S // CH
LN_EPS = 1e-5
NEG = -1e9
QSCALE = (DH ** -0.5) * 1.4426950408889634

_NT = (((1,), (1,)), ((), ()))
_NN = (((1,), (0,)), ((), ()))
_TN = (((0,), (0,)), ((), ()))


def _kernel(x_hbm, wqkv_hbm, wo_hbm, wr_ref, wg_hbm, wu_hbm, wd_hbm,
            o_ref,
            x_ref, wqkv_ref, wo_ref, wg_ref, wu_ref, wd_ref, wqt_s, wvt_s,
            xn_s, q_s, k_s, vt_s, y_s, ot_s, sa_s, sb_s, idx_s, sems):
    I = pl.program_id(0)
    f32 = jnp.float32
    bf16 = jnp.bfloat16

    @pl.when(I == 0)
    def _prologue():
        wr = wr_ref[...].astype(f32).reshape(1, D)

        def x_copy(c):
            r0 = pl.multiple_of(c * CH, CH)
            return pltpu.make_async_copy(x_hbm.at[pl.ds(r0, CH)], x_ref.at[pl.ds(r0, CH)],
                                         sems.at[c])
        def w_part(j):
            return pltpu.make_async_copy(wqkv_hbm.at[:, pl.ds(j * D, D)],
                                         wqkv_ref.at[:, pl.ds(j * D, D)], sems.at[NC + 5 + j])
        wo_cp = pltpu.make_async_copy(wo_hbm, wo_ref, sems.at[NC + 1])
        wg_cp = pltpu.make_async_copy(wg_hbm, wg_ref, sems.at[NC + 2])
        wu_cp = pltpu.make_async_copy(wu_hbm, wu_ref, sems.at[NC + 3])
        wd_cp = pltpu.make_async_copy(wd_hbm, wd_ref, sems.at[NC + 4])
        x_copy(0).start()
        w_part(1).start()
        w_part(0).start()
        w_part(2).start()
        for c in range(1, NC):
            x_copy(c).start()
        wo_cp.start()
        wg_cp.start()
        wu_cp.start()
        wd_cp.start()

        def ln_chunk(c, carry):
            best_val, best_idx = carry
            r0 = pl.multiple_of(c * CH, CH)
            xc = x_ref[pl.ds(r0, CH), :].astype(f32)
            m = jnp.mean(xc, axis=-1, keepdims=True)
            xc0 = xc - m
            v = jnp.mean(xc0 * xc0, axis=-1, keepdims=True)
            xn = (xc0 * lax.rsqrt(v + LN_EPS)).astype(bf16)
            xn_s[pl.ds(r0, CH), :] = xn
            r = jnp.sum(xn.astype(f32) * wr, axis=-1, keepdims=True)
            r = r.astype(bf16).astype(f32)
            cmax = jnp.max(r)
            rows = lax.broadcasted_iota(jnp.int32, (CH, 1), 0) + r0
            cidx = jnp.min(jnp.where(r == cmax, rows, S))
            better = cmax > best_val
            best_idx = jnp.where(better, cidx, best_idx)
            best_val = jnp.where(better, cmax, best_val)
            return best_val, best_idx

        def k_proj(c):
            r0 = pl.multiple_of(c * CH, CH)
            k = jnp.dot(xn_s[pl.ds(r0, CH), :], wqkv_ref[:, D:2 * D], preferred_element_type=f32)
            k_s[pl.ds(r0, CH), :] = k.astype(bf16)

        def qv_proj(c):
            r0 = pl.multiple_of(c * CH, CH)
            xn = xn_s[pl.ds(r0, CH), :]
            qt = lax.dot_general(wqt_s[...], xn, _NT, preferred_element_type=f32)
            q_s[:, pl.ds(r0, CH)] = (qt * QSCALE).astype(bf16)
            vt = lax.dot_general(wvt_s[...], xn, _NT, preferred_element_type=f32)
            vt_s[:, pl.ds(r0, CH)] = vt.astype(bf16)

        def proj_chunk(c):
            k_proj(c)
            qv_proj(c)

        x_copy(0).wait()
        best = ln_chunk(0, (jnp.float32(-jnp.inf), jnp.int32(0)))
        w_part(1).wait()
        k_proj(0)
        w_part(0).wait()
        w_part(2).wait()
        wqt_s[...] = wqkv_ref[:, 0:D].T
        wvt_s[...] = wqkv_ref[:, 2 * D:3 * D].T
        x_copy(1).wait()
        best = ln_chunk(1, best)
        qv_proj(0)

        def body(c, best):
            x_copy(c + 1).wait()
            best = ln_chunk(c + 1, best)
            proj_chunk(c)
            return best

        best_val, best_idx = lax.fori_loop(1, NC - 1, body, best)
        idx_s[0] = best_idx
        wo_cp.wait()
        wg_cp.wait()
        wu_cp.wait()
        wd_cp.wait()

        base = pl.multiple_of((best_idx // 16) * 16, 16)
        slab = xn_s[pl.ds(base, 16), :].astype(f32)
        rows16 = lax.broadcasted_iota(jnp.int32, (16, D), 0) + base
        xsel = jnp.sum(jnp.where(rows16 == best_idx, slab, 0.0), axis=0, keepdims=True)
        xsel8 = jnp.broadcast_to(xsel, (8, D)).astype(bf16)
        g = lax.dot_general(xsel8, wg_ref[...], _NT, preferred_element_type=f32)
        g = g.astype(bf16).astype(f32)
        g = (g * jax.nn.sigmoid(g)).astype(bf16).astype(f32)
        u = lax.dot_general(xsel8, wu_ref[...], _NT, preferred_element_type=f32)
        u = u.astype(bf16).astype(f32)
        hmid = (g * u).astype(bf16)
        y = jnp.dot(hmid, wd_ref[...], preferred_element_type=f32)
        y = y.astype(bf16).astype(f32)
        rsel = jax.nn.sigmoid(best_val).astype(bf16).astype(f32)
        y_s[...] = (y * rsel).astype(bf16).astype(f32)

        proj_chunk(NC - 1)

    r0 = pl.multiple_of(I * BQ, BQ)
    row = lax.broadcasted_iota(jnp.int32, (BQ, BQ), 0)
    col = lax.broadcasted_iota(jnp.int32, (BQ, BQ), 1)
    tri = row <= col

    def attention(ntiles):
        def koff(t):
            return pl.multiple_of((I - 2 + t) * BQ, BQ)

        def stage_a(j, sbuf):
            g, a0 = j // 2, (j % 2) * 4
            cols = []
            for u in range(4):
                a = a0 + u
                h = g * 8 + a
                parts = []
                if a > 0:
                    parts.append(jnp.zeros((a * DH, BQ), bf16))
                parts.append(q_s[pl.ds(h * DH, DH), pl.ds(r0, BQ)])
                if a < 7:
                    parts.append(jnp.zeros(((7 - a) * DH, BQ), bf16))
                cols.append(jnp.concatenate(parts, axis=0))
            wq = jnp.concatenate(cols, axis=1)
            ksl = lambda t: k_s[pl.ds(koff(t), BQ), g * 128:(g + 1) * 128]
            st2 = jnp.dot(ksl(2), wq, preferred_element_type=f32)
            st0 = jnp.dot(ksl(0), wq, preferred_element_type=f32) if ntiles == 3 else None
            ms = []
            for u in range(4):
                sl = slice(u * BQ, (u + 1) * BQ)
                other = st0[:, sl] if ntiles == 3 else NEG
                sm = jnp.where(tri, st2[:, sl], other)
                sbuf[0:BQ, sl] = sm
                ms.append(jnp.max(sm, axis=0, keepdims=True))
            m = jnp.concatenate(ms, axis=1)
            if ntiles >= 2:
                st1 = jnp.dot(ksl(1), wq, preferred_element_type=f32)
                sbuf[BQ:2 * BQ, :] = st1
                m = jnp.maximum(m, jnp.max(st1, axis=0, keepdims=True))
            return m

        def stage_b(j, sbuf, m):
            g, a0 = j // 2, (j % 2) * 4
            for u in range(4):
                h = g * 8 + a0 + u
                sl = slice(u * BQ, (u + 1) * BQ)
                mu = m[:, sl]
                vsl = lambda t: vt_s[pl.ds(h * DH, DH), pl.ds(koff(t), BQ)]
                pm = jnp.exp2(sbuf[0:BQ, sl] - mu)
                l = jnp.sum(pm, axis=0, keepdims=True)
                if ntiles == 3:
                    ot = jnp.dot(vsl(2), jnp.where(tri, pm, 0.0).astype(bf16),
                                 preferred_element_type=f32)
                    ot = ot + jnp.dot(vsl(0), jnp.where(tri, 0.0, pm).astype(bf16),
                                      preferred_element_type=f32)
                else:
                    ot = jnp.dot(vsl(2), pm.astype(bf16), preferred_element_type=f32)
                if ntiles >= 2:
                    p1 = jnp.exp2(sbuf[BQ:2 * BQ, sl] - mu)
                    l = l + jnp.sum(p1, axis=0, keepdims=True)
                    ot = ot + jnp.dot(vsl(1), p1.astype(bf16), preferred_element_type=f32)
                ot_s[pl.ds(h * DH, DH), pl.ds(pl.multiple_of((I % 2) * BQ, BQ), BQ)] = (ot / l).astype(bf16)

        bufs = (sa_s, sb_s)
        NQ = 8
        m_prev = stage_a(0, bufs[0])
        for j in range(NQ):
            m_next = stage_a(j + 1, bufs[(j + 1) % 2]) if j + 1 < NQ else None
            stage_b(j, bufs[j % 2], m_prev)
            m_prev = m_next

    @pl.when(I >= 2)
    def _():
        attention(3)

    @pl.when(I == 1)
    def _():
        attention(2)

    @pl.when(I == 0)
    def _():
        attention(1)

    @pl.when(I % 2 == 1)
    def _epilogue():
        r2 = pl.multiple_of((I - 1) * BQ, 2 * BQ)
        att = lax.dot_general(ot_s[...], wo_ref[...], _TN,
                              preferred_element_type=f32)
        xb = x_ref[pl.ds(r2, 2 * BQ), :].astype(f32)
        xnb = xn_s[pl.ds(r2, 2 * BQ), :].astype(f32)
        rows = lax.broadcasted_iota(jnp.int32, (2 * BQ, D), 0) + r2
        upd = jnp.where(rows == idx_s[0], jnp.broadcast_to(y_s[0:1, :], (2 * BQ, D)), 0.0)
        o_ref[...] = (xb + att + (xnb + upd)).astype(o_ref.dtype)


@jax.jit
def pallas_parallel_sum__sliding_block__moe_arch_mod__prompt_kernel(
    A_x: jax.Array,
    A_wqkv: jax.Array,
    A_wo: jax.Array,
    B_x: jax.Array,
    B_w_r: jax.Array,
    B_w_gate: jax.Array,
    B_w_up: jax.Array,
    B_w_down: jax.Array,
):
    del B_x
    x = A_x.reshape(S, D)
    wr = B_w_r
    bf16 = jnp.bfloat16
    f32 = jnp.float32
    any_spec = pl.BlockSpec(memory_space=pl.ANY)
    out = pl.pallas_call(
        _kernel,
        grid=(NB,),
        in_specs=[
            any_spec,
            any_spec,
            any_spec,
            pl.BlockSpec((D,), lambda i: (0,)),
            any_spec,
            any_spec,
            any_spec,
        ],
        out_specs=pl.BlockSpec((2 * BQ, D), lambda i: (i // 2, 0)),
        out_shape=jax.ShapeDtypeStruct((S, D), A_x.dtype),
        scratch_shapes=[
            pltpu.VMEM((S, D), bf16),
            pltpu.VMEM((D, 3 * D), bf16),
            pltpu.VMEM((D, D), bf16),
            pltpu.VMEM((F, D), bf16),
            pltpu.VMEM((F, D), bf16),
            pltpu.VMEM((F, D), bf16),
            pltpu.VMEM((D, D), bf16),
            pltpu.VMEM((D, D), bf16),
            pltpu.VMEM((S, D), bf16),
            pltpu.VMEM((D, S), bf16),
            pltpu.VMEM((S, D), bf16),
            pltpu.VMEM((D, S), bf16),
            pltpu.VMEM((8, D), f32),
            pltpu.VMEM((D, 2 * BQ), bf16),
            pltpu.VMEM((2 * BQ, 4 * BQ), f32),
            pltpu.VMEM((2 * BQ, 4 * BQ), f32),
            pltpu.SMEM((1,), jnp.int32),
            pltpu.SemaphoreType.DMA((NC + 8,)),
        ],
        compiler_params=pltpu.CompilerParams(
            dimension_semantics=("arbitrary",),
            vmem_limit_bytes=100 * 1024 * 1024,
        ),
    )(x, A_wqkv, A_wo, wr, B_w_gate.T, B_w_up.T, B_w_down)
    return out.reshape(A_x.shape)
```

```python
import jax
import jax.numpy as jnp
from jax import lax
import jax.experimental.pallas as pl
import jax.experimental.pallas.tpu as pltpu

S = 2048
D = 512
H = 32
DH = 16
W = 256
F = 1376
BQ = 128
NB = S // BQ
BPS = 4
CH = 512
NC = S // CH
LN_EPS = 1e-5
NEG = -1e9
QSCALE = (DH ** -0.5) * 1.4426950408889634

_NT = (((1,), (1,)), ((), ()))
_NN = (((1,), (0,)), ((), ()))
_TN = (((0,), (0,)), ((), ()))
_TT = (((0,), (1,)), ((), ()))


def _kernel(x_hbm, wqkv_hbm, wo_hbm, wr_ref, wg_hbm, wu_hbm, wd_hbm,
            o_ref,
            x_ref, wqkv_ref, wo_ref, wg_ref, wu_ref, wd_ref,
            xn_s, q_s, k_s, vt_s, y_s, ot_s, sa_s, sb_s, idx_s, sems):
    I = pl.program_id(0)
    f32 = jnp.float32
    bf16 = jnp.bfloat16

    @pl.when(I == 0)
    def _prologue():
        wr = wr_ref[...].astype(f32).reshape(1, D)

        def x_copy(c):
            r0 = pl.multiple_of(c * CH, CH)
            return pltpu.make_async_copy(x_hbm.at[pl.ds(r0, CH)], x_ref.at[pl.ds(r0, CH)],
                                         sems.at[c])
        def w_part(j):
            return pltpu.make_async_copy(wqkv_hbm.at[:, pl.ds(j * D, D)],
                                         wqkv_ref.at[:, pl.ds(j * D, D)], sems.at[NC + 5 + j])
        wo_cp = pltpu.make_async_copy(wo_hbm, wo_ref, sems.at[NC + 1])
        wg_cp = pltpu.make_async_copy(wg_hbm, wg_ref, sems.at[NC + 2])
        wu_cp = pltpu.make_async_copy(wu_hbm, wu_ref, sems.at[NC + 3])
        wd_cp = pltpu.make_async_copy(wd_hbm, wd_ref, sems.at[NC + 4])
        x_copy(0).start()
        w_part(1).start()
        w_part(0).start()
        w_part(2).start()
        for c in range(1, NC):
            x_copy(c).start()
        wo_cp.start()
        wg_cp.start()
        wu_cp.start()
        wd_cp.start()

        def ln_chunk(c, carry):
            best_val, best_idx = carry
            r0 = pl.multiple_of(c * CH, CH)
            xc = x_ref[pl.ds(r0, CH), :].astype(f32)
            m = jnp.mean(xc, axis=-1, keepdims=True)
            xc0 = xc - m
            v = jnp.mean(xc0 * xc0, axis=-1, keepdims=True)
            xn = (xc0 * lax.rsqrt(v + LN_EPS)).astype(bf16)
            xn_s[pl.ds(r0, CH), :] = xn
            r = jnp.sum(xn.astype(f32) * wr, axis=-1, keepdims=True)
            r = r.astype(bf16).astype(f32)
            cmax = jnp.max(r)
            rows = lax.broadcasted_iota(jnp.int32, (CH, 1), 0) + r0
            cidx = jnp.min(jnp.where(r == cmax, rows, S))
            better = cmax > best_val
            best_idx = jnp.where(better, cidx, best_idx)
            best_val = jnp.where(better, cmax, best_val)
            return best_val, best_idx

        def k_proj(c):
            r0 = pl.multiple_of(c * CH, CH)
            k = jnp.dot(xn_s[pl.ds(r0, CH), :], wqkv_ref[:, D:2 * D], preferred_element_type=f32)
            k_s[pl.ds(r0, CH), :] = k.astype(bf16)

        def qv_proj(c):
            r0 = pl.multiple_of(c * CH, CH)
            xn = xn_s[pl.ds(r0, CH), :]
            qt = lax.dot_general(wqkv_ref[:, 0:D], xn, _TT, preferred_element_type=f32)
            q_s[:, pl.ds(r0, CH)] = (qt * QSCALE).astype(bf16)
            vt = lax.dot_general(wqkv_ref[:, 2 * D:3 * D], xn, _TT, preferred_element_type=f32)
            vt_s[:, pl.ds(r0, CH)] = vt.astype(bf16)

        def proj_chunk(c):
            k_proj(c)
            qv_proj(c)

        x_copy(0).wait()
        best = ln_chunk(0, (jnp.float32(-jnp.inf), jnp.int32(0)))
        w_part(1).wait()
        k_proj(0)
        w_part(0).wait()
        w_part(2).wait()
        x_copy(1).wait()
        best = ln_chunk(1, best)
        qv_proj(0)

        def body(c, best):
            x_copy(c + 1).wait()
            best = ln_chunk(c + 1, best)
            proj_chunk(c)
            return best

        best_val, best_idx = lax.fori_loop(1, NC - 1, body, best)
        idx_s[0] = best_idx
        wo_cp.wait()
        wg_cp.wait()
        wu_cp.wait()
        wd_cp.wait()

        base = pl.multiple_of((best_idx // 16) * 16, 16)
        slab = xn_s[pl.ds(base, 16), :].astype(f32)
        rows16 = lax.broadcasted_iota(jnp.int32, (16, D), 0) + base
        xsel = jnp.sum(jnp.where(rows16 == best_idx, slab, 0.0), axis=0, keepdims=True)
        xsel8 = jnp.broadcast_to(xsel, (8, D)).astype(bf16)
        g = lax.dot_general(xsel8, wg_ref[...], _NT, preferred_element_type=f32)
        g = g.astype(bf16).astype(f32)
        g = (g * jax.nn.sigmoid(g)).astype(bf16).astype(f32)
        u = lax.dot_general(xsel8, wu_ref[...], _NT, preferred_element_type=f32)
        u = u.astype(bf16).astype(f32)
        hmid = (g * u).astype(bf16)
        y = jnp.dot(hmid, wd_ref[...], preferred_element_type=f32)
        y = y.astype(bf16).astype(f32)
        rsel = jax.nn.sigmoid(best_val).astype(bf16).astype(f32)
        y_s[...] = (y * rsel).astype(bf16).astype(f32)

        proj_chunk(NC - 1)

    row = lax.broadcasted_iota(jnp.int32, (BQ, BQ), 0)
    col = lax.broadcasted_iota(jnp.int32, (BQ, BQ), 1)
    tri = row <= col

    def stage_a(blk, ntiles, j, sbuf):
        koff = lambda t: pl.multiple_of((blk - 2 + t) * BQ, BQ)
        rq = pl.multiple_of(blk * BQ, BQ)
        g, a0 = j // 2, (j % 2) * 4
        cols = []
        for u in range(4):
            a = a0 + u
            h = g * 8 + a
            parts = []
            if a > 0:
                parts.append(jnp.zeros((a * DH, BQ), bf16))
            parts.append(q_s[pl.ds(h * DH, DH), pl.ds(rq, BQ)])
            if a < 7:
                parts.append(jnp.zeros(((7 - a) * DH, BQ), bf16))
            cols.append(jnp.concatenate(parts, axis=0))
        wq = jnp.concatenate(cols, axis=1)
        ksl = lambda t: k_s[pl.ds(koff(t), BQ), g * 128:(g + 1) * 128]
        st2 = jnp.dot(ksl(2), wq, preferred_element_type=f32)
        st0 = jnp.dot(ksl(0), wq, preferred_element_type=f32) if ntiles == 3 else None
        ms = []
        for u in range(4):
            sl = slice(u * BQ, (u + 1) * BQ)
            other = st0[:, sl] if ntiles == 3 else NEG
            sm = jnp.where(tri, st2[:, sl], other)
            sbuf[0:BQ, sl] = sm
            ms.append(jnp.max(sm, axis=0, keepdims=True))
        m = jnp.concatenate(ms, axis=1)
        if ntiles >= 2:
            st1 = jnp.dot(ksl(1), wq, preferred_element_type=f32)
            sbuf[BQ:2 * BQ, :] = st1
            m = jnp.maximum(m, jnp.max(st1, axis=0, keepdims=True))
        return m

    def stage_b(blk, ntiles, s, j, sbuf, m):
        koff = lambda t: pl.multiple_of((blk - 2 + t) * BQ, BQ)
        g, a0 = j // 2, (j % 2) * 4
        for u in range(4):
            h = g * 8 + a0 + u
            sl = slice(u * BQ, (u + 1) * BQ)
            mu = m[:, sl]
            vsl = lambda t: vt_s[pl.ds(h * DH, DH), pl.ds(koff(t), BQ)]
            pm = jnp.exp2(sbuf[0:BQ, sl] - mu)
            l = jnp.sum(pm, axis=0, keepdims=True)
            if ntiles == 3:
                ot = jnp.dot(vsl(2), jnp.where(tri, pm, 0.0).astype(bf16),
                             preferred_element_type=f32)
                ot = ot + jnp.dot(vsl(0), jnp.where(tri, 0.0, pm).astype(bf16),
                                  preferred_element_type=f32)
            else:
                ot = jnp.dot(vsl(2), pm.astype(bf16), preferred_element_type=f32)
            if ntiles >= 2:
                p1 = jnp.exp2(sbuf[BQ:2 * BQ, sl] - mu)
                l = l + jnp.sum(p1, axis=0, keepdims=True)
                ot = ot + jnp.dot(vsl(1), p1.astype(bf16), preferred_element_type=f32)
            ot_s[pl.ds(h * DH, DH), s * BQ:(s + 1) * BQ] = (ot / l).astype(bf16)

    def attention(nts):
        units = [(s, j) for s in range(BPS) for j in range(8)]
        bufs = (sa_s, sb_s)
        blk = lambda s: BPS * I + s
        m_prev = stage_a(blk(0), nts[0], 0, bufs[0])
        for k, (s, j) in enumerate(units):
            if k + 1 < len(units):
                s2, j2 = units[k + 1]
                m_next = stage_a(blk(s2), nts[s2], j2, bufs[(k + 1) % 2])
            else:
                m_next = None
            stage_b(blk(s), nts[s], s, j, bufs[k % 2], m_prev)
            m_prev = m_next

    @pl.when(I == 0)
    def _():
        attention((1, 2) + (3,) * (BPS - 2))

    @pl.when(I >= 1)
    def _():
        attention((3,) * BPS)

    RB = BPS * BQ
    EP = 256
    for e in range(RB // EP):
        r2 = pl.multiple_of(I * RB + e * EP, EP)
        att = lax.dot_general(ot_s[:, e * EP:(e + 1) * EP], wo_ref[...], _TN,
                              preferred_element_type=f32)
        xb = x_ref[pl.ds(r2, EP), :].astype(f32)
        xnb = xn_s[pl.ds(r2, EP), :].astype(f32)
        rows = lax.broadcasted_iota(jnp.int32, (EP, D), 0) + r2
        upd = jnp.where(rows == idx_s[0], jnp.broadcast_to(y_s[0:1, :], (EP, D)), 0.0)
        o_ref[e * EP:(e + 1) * EP, :] = (xb + att + (xnb + upd)).astype(o_ref.dtype)


@jax.jit
def pallas_parallel_sum__sliding_block__moe_arch_mod__prompt_kernel(
    A_x: jax.Array,
    A_wqkv: jax.Array,
    A_wo: jax.Array,
    B_x: jax.Array,
    B_w_r: jax.Array,
    B_w_gate: jax.Array,
    B_w_up: jax.Array,
    B_w_down: jax.Array,
):
    del B_x
    x = A_x.reshape(S, D)
    wr = B_w_r
    bf16 = jnp.bfloat16
    f32 = jnp.float32
    any_spec = pl.BlockSpec(memory_space=pl.ANY)
    out = pl.pallas_call(
        _kernel,
        grid=(NB // BPS,),
        in_specs=[
            any_spec,
            any_spec,
            any_spec,
            pl.BlockSpec((D,), lambda i: (0,)),
            any_spec,
            any_spec,
            any_spec,
        ],
        out_specs=pl.BlockSpec((BPS * BQ, D), lambda i: (i, 0)),
        out_shape=jax.ShapeDtypeStruct((S, D), A_x.dtype),
        scratch_shapes=[
            pltpu.VMEM((S, D), bf16),
            pltpu.VMEM((D, 3 * D), bf16),
            pltpu.VMEM((D, D), bf16),
            pltpu.VMEM((F, D), bf16),
            pltpu.VMEM((F, D), bf16),
            pltpu.VMEM((F, D), bf16),
            pltpu.VMEM((S, D), bf16),
            pltpu.VMEM((D, S), bf16),
            pltpu.VMEM((S, D), bf16),
            pltpu.VMEM((D, S), bf16),
            pltpu.VMEM((8, D), f32),
            pltpu.VMEM((D, BPS * BQ), bf16),
            pltpu.VMEM((2 * BQ, 4 * BQ), f32),
            pltpu.VMEM((2 * BQ, 4 * BQ), f32),
            pltpu.SMEM((1,), jnp.int32),
            pltpu.SemaphoreType.DMA((NC + 8,)),
        ],
        compiler_params=pltpu.CompilerParams(
            dimension_semantics=("arbitrary",),
            vmem_limit_bytes=100 * 1024 * 1024,
        ),
    )(x, A_wqkv, A_wo, wr, B_w_gate.T, B_w_up.T, B_w_down)
    return out.reshape(A_x.shape)
```
